```python
import jax
import jax.numpy as jnp

def _softmax(x, axis=-1):
    return jax.nn.softmax(x, axis=axis)

def _gelu(x):
    return jax.nn.gelu(x, approximate=True)

def _silu(x):
    return jax.nn.silu(x)

def _sigmoid(x):
    return jax.nn.sigmoid(x)

def _layernorm(x, axis=-1, eps=1e-05):
    m = jnp.mean(x, axis=axis, keepdims=True)
    v = jnp.var(x, axis=axis, keepdims=True)
    return (x - m) / jnp.sqrt(v + eps)

def _scatter_add(tgt, idx, src, axis=0):
    return tgt.at[idx].add(src)

def _segment_sum(src, seg, n):
    return jax.ops.segment_sum(src, seg, n)

class _Rng:

    def __init__(self, key):
        self._k = key

    def _next(self):
        self._k, sub = jax.random.split(self._k)
        return sub

    def normal(self, shape):
        return jax.random.normal(self._next(), shape, dtype=jnp.bfloat16)

    def randint(self, lo, hi, shape):
        return jax.random.randint(self._next(), shape, lo, hi, dtype=jnp.int32)

    def uniform(self, shape, lo=0.0, hi=1.0):
        return jax.random.uniform(self._next(), shape, jnp.bfloat16, lo, hi)

    def permutation(self, n):
        return jax.random.permutation(self._next(), n)
kernel_name = 'adaLN_cond__sliding_block_cached__glu_gated_bilinear__decode'

def setup_inputs():
    _rng = _Rng(jax.random.key(int.from_bytes(__import__("os").urandom(4), "little")))
    _w = lambda a: (lambda t: t.astype(jnp.bfloat16) if jnp.issubdtype(t.dtype, jnp.floating) else t)(jnp.asarray(a))

    def _A_setup():
        B, Sq, D = (1, 1, 640)
        Hq, Hkv, Sk, Dh = (32, 32, 32768, 192)
        assert Hq % Hkv == 0, (Hq, Hkv)
        return {'x': _w((lambda *s: _rng.normal(s) * 0.05)(B, Sq, D)), 'k_cache': _w((lambda *s: _rng.normal(s) * 0.05)(B, Hkv, Sk, Dh)), 'v_cache': _w((lambda *s: _rng.normal(s) * 0.05)(B, Hkv, Sk, Dh)), 'wq': _w((lambda *s: _rng.normal(s) * 0.05)(D, Hq * Dh) * D ** (-0.5)), 'wo': _w((lambda *s: _rng.normal(s) * 0.05)(Hq * Dh, D) * (Hq * Dh) ** (-0.5))}
    _A_in = _A_setup()

    def _B_setup():
        B, S, D, F = (1, 1, 640, 1536)
        return {'x': _w((lambda *s: _rng.normal(s) * 0.05)(B, S, D)), 'w_gate': _w((lambda *s: _rng.normal(s) * 0.05)(D, F) * D ** (-0.5)), 'w_up': _w((lambda *s: _rng.normal(s) * 0.05)(D, F) * D ** (-0.5)), 'w_down': _w((lambda *s: _rng.normal(s) * 0.05)(F, D) * F ** (-0.5))}
    _B_in = _B_setup()
    return {'A_x': _A_in['x'], 'A_k_cache': _A_in['k_cache'], 'A_v_cache': _A_in['v_cache'], 'A_wq': _A_in['wq'], 'A_wo': _A_in['wo'], 'B_x': _B_in['x'], 'B_w_gate': _B_in['w_gate'], 'B_w_up': _B_in['w_up'], 'B_w_down': _B_in['w_down'], 'c': _w((lambda *s: _rng.normal(s) * 0.05)(1, 640)), 'w_mod': _w((lambda *s: _rng.normal(s) * 0.05)(640, 6 * 640) * 640 ** (-0.5))}

def reference(A_x, A_k_cache, A_v_cache, A_wq, A_wo, B_x, B_w_gate, B_w_up, B_w_down, c, w_mod):

    def _A_ref(x, k_cache, v_cache, wq, wo):
        B, Sq, D = x.shape
        Hq, Dh = (32, 192)
        Hkv, Sk = (k_cache.shape[1], k_cache.shape[2])
        W = min(4096, max(256, Sk // 4))
        rep = Hq // Hkv
        q = (lambda x, *d: x.transpose(*d))((x @ wq).reshape(B, Sq, Hq, Dh), 0, 2, 1, 3)
        k = jnp.repeat(k_cache[:, :, Sk - W:, :], rep, axis=1)
        v = jnp.repeat(v_cache[:, :, Sk - W:, :], rep, axis=1)
        scores = jnp.einsum('bhqd,bhkd->bhqk', q, k) * Dh ** (-0.5)
        p = _softmax(scores, axis=-1)
        o = jnp.einsum('bhqk,bhkd->bhqd', p, v)
        return (lambda x, *d: x.transpose(*d))(o, 0, 2, 1, 3).reshape(B, Sq, Hq * Dh) @ wo

    def _B_ref(x, w_gate, w_up, w_down):
        g = jnp.einsum('bsd,df->bsf', x, w_gate)
        u = jnp.einsum('bsd,df->bsf', x, w_up)
        h = g * u
        return jnp.einsum('bsf,fd->bsd', h, w_down)
    x = A_x
    mod = (_silu(c) @ w_mod).reshape(c.shape[0], 6, 1, -1)
    sa, ca, ga, sb, cb, gb = (mod[:, 0].copy(), mod[:, 1].copy(), mod[:, 2].copy(), mod[:, 3].copy(), mod[:, 4].copy(), mod[:, 5].copy())
    h = _layernorm(x, axis=-1) * (1 + ca) + sa
    x = x + ga * _A_ref(h, A_k_cache, A_v_cache, A_wq, A_wo)
    h = _layernorm(x, axis=-1) * (1 + cb) + sb
    x = x + gb * _B_ref(h, B_w_gate, B_w_up, B_w_down)
    return x
```

```python
import jax
import jax.numpy as jnp
import jax.experimental.pallas as pl
import jax.experimental.pallas.tpu as pltpu

D = 640
H = 32
DH = 192
F = 1536
M = 8
NS = 2
FCH = 3
PR = 2 * DH
NP = H * DH // PR


def _kernel(x_hbm, k_hbm, v_hbm, wq_hbm, wo_hbm, wg_hbm, wu_hbm, wd_hbm, c_hbm, wm_hbm,
            o_ref,
            x_v, c_v, kbuf, vbuf, wq_v, wo_v, wg_v, wu_v, wd_v, wm_v, q_s,
            ksem, vsem, wsem):
    SK = k_hbm.shape[1]
    W = kbuf.shape[2]
    c0 = SK - W

    def kcopy(p, slot):
        return pltpu.make_async_copy(
            k_hbm.at[pl.ds(pl.multiple_of(p * PR, PR), PR), pl.ds(c0, W)], kbuf.at[slot], ksem.at[slot])

    def vcopy(p, slot):
        return pltpu.make_async_copy(
            v_hbm.at[pl.ds(pl.multiple_of(p * PR, PR), PR), pl.ds(c0, W)], vbuf.at[slot], vsem.at[slot])

    x_cp = pltpu.make_async_copy(x_hbm, x_v, wsem.at[0])
    c_cp = pltpu.make_async_copy(c_hbm, c_v, wsem.at[1])
    wm_cp = pltpu.make_async_copy(wm_hbm, wm_v, wsem.at[2])
    wq_cp = pltpu.make_async_copy(wq_hbm, wq_v, wsem.at[3])
    wo_cp = pltpu.make_async_copy(wo_hbm, wo_v, wsem.at[4])
    FC = F // FCH
    g_cp = [pltpu.make_async_copy(wg_hbm.at[:, pl.ds(i * FC, FC)], wg_v.at[:, pl.ds(i * FC, FC)], wsem.at[5 + i])
            for i in range(FCH)]
    u_cp = [pltpu.make_async_copy(wu_hbm.at[:, pl.ds(i * FC, FC)], wu_v.at[:, pl.ds(i * FC, FC)], wsem.at[5 + FCH + i])
            for i in range(FCH)]
    d_cp = [pltpu.make_async_copy(wd_hbm.at[pl.ds(i * FC, FC), :], wd_v.at[pl.ds(i * FC, FC), :], wsem.at[5 + 2 * FCH + i])
            for i in range(FCH)]

    c_cp.start()
    wm_cp.start()
    x_cp.start()
    wq_cp.start()
    wo_cp.start()
    for s in range(NS):
        kcopy(s, s).start()
        vcopy(s, s).start()

    c_cp.wait()
    cf = c_v[...].astype(jnp.float32)
    sc = cf * jax.nn.sigmoid(cf)
    sc = jnp.broadcast_to(sc, (M, D)).astype(jnp.bfloat16)
    wm_cp.wait()
    mod = jnp.dot(sc, wm_v[...], preferred_element_type=jnp.float32)
    sa = mod[:, 0 * D:1 * D]
    ca = mod[:, 1 * D:2 * D]
    ga = mod[:, 2 * D:3 * D]
    sb = mod[:, 3 * D:4 * D]
    cb = mod[:, 4 * D:5 * D]
    gb = mod[:, 5 * D:6 * D]

    def ln(t):
        m = jnp.mean(t, axis=-1, keepdims=True)
        d = t - m
        v = jnp.mean(d * d, axis=-1, keepdims=True)
        return d * jax.lax.rsqrt(v + 1e-5)

    x_cp.wait()
    x = jnp.broadcast_to(x_v[...].astype(jnp.float32), (M, D))
    h = (ln(x) * (1.0 + ca) + sa).astype(jnp.bfloat16)
    wq_cp.wait()
    row = jax.lax.broadcasted_iota(jnp.int32, (M, PR), 0)
    col = jax.lax.broadcasted_iota(jnp.int32, (M, PR), 1)
    hmask = ((row == 0) & (col < DH)) | ((row == 1) & (col >= DH))
    scale = DH ** -0.5
    for p in range(NP):
        q = jnp.dot(h, wq_v[:, p * PR:(p + 1) * PR], preferred_element_type=jnp.float32)
        q_s[p] = jnp.where(hmask, q * scale, 0.0).astype(jnp.bfloat16)
    wo_cp.wait()

    def body(p, acc):
        slot = p % NS
        kcopy(p, slot).wait()
        s = jnp.dot(q_s[p], kbuf[slot], preferred_element_type=jnp.float32)

        @pl.when(p + NS < NP)
        def _():
            kcopy(p + NS, slot).start()

        m = jnp.max(s, axis=-1, keepdims=True)
        e = jnp.exp(s - m)
        l = jnp.sum(e, axis=-1, keepdims=True)
        vcopy(p, slot).wait()
        o = jax.lax.dot_general(e.astype(jnp.bfloat16), vbuf[slot], (((1,), (1,)), ((), ())),
                                preferred_element_type=jnp.float32)

        @pl.when(p + NS < NP)
        def _():
            vcopy(p + NS, slot).start()

        @pl.when(p + NS == NP)
        def _():
            for i in range(FCH):
                g_cp[i].start()
                u_cp[i].start()
            for i in range(FCH):
                d_cp[i].start()

        on = jnp.where(hmask, o / l, 0.0).astype(jnp.bfloat16)
        return acc + jnp.dot(on, wo_v[pl.ds(pl.multiple_of(p * PR, PR), PR), :], preferred_element_type=jnp.float32)

    acc = jax.lax.fori_loop(0, NP, body, jnp.zeros((M, D), jnp.float32))
    attn = jnp.sum(acc, axis=0, keepdims=True)
    x1 = x + ga * attn
    h2 = (ln(x1) * (1.0 + cb) + sb).astype(jnp.bfloat16)
    hs = []
    for i in range(FCH):
        g_cp[i].wait()
        g = jnp.dot(h2, wg_v[:, i * FC:(i + 1) * FC], preferred_element_type=jnp.float32)
        u_cp[i].wait()
        u = jnp.dot(h2, wu_v[:, i * FC:(i + 1) * FC], preferred_element_type=jnp.float32)
        hs.append((g * u).astype(jnp.bfloat16))
    y = jnp.zeros((M, D), jnp.float32)
    for i in range(FCH):
        d_cp[i].wait()
        y = y + jnp.dot(hs[i], wd_v[i * FC:(i + 1) * FC, :], preferred_element_type=jnp.float32)
    out = x1 + gb * y
    o_ref[...] = out[0:1, :].astype(o_ref.dtype)


@jax.jit
def pallas_adaLN_cond__sliding_block_cached__glu_gated_bilinear__decode_kernel(
    A_x: jax.Array,
    A_k_cache: jax.Array,
    A_v_cache: jax.Array,
    A_wq: jax.Array,
    A_wo: jax.Array,
    B_x: jax.Array,
    B_w_gate: jax.Array,
    B_w_up: jax.Array,
    B_w_down: jax.Array,
    c: jax.Array,
    w_mod: jax.Array,
):
    B, Hkv, SK, Dh = A_k_cache.shape
    W = min(4096, max(256, SK // 4))
    kt = jnp.transpose(A_k_cache, (0, 1, 3, 2)).reshape(Hkv * Dh, SK)
    vt = jnp.transpose(A_v_cache, (0, 1, 3, 2)).reshape(Hkv * Dh, SK)
    x2 = A_x.reshape(1, D)
    anyspec = pl.BlockSpec(memory_space=pl.ANY)
    out = pl.pallas_call(
        _kernel,
        in_specs=[anyspec] * 10,
        out_specs=pl.BlockSpec(memory_space=pltpu.VMEM),
        out_shape=jax.ShapeDtypeStruct((1, D), A_x.dtype),
        scratch_shapes=[
            pltpu.VMEM((1, D), jnp.bfloat16),
            pltpu.VMEM((1, D), jnp.bfloat16),
            pltpu.VMEM((NS, PR, W), jnp.bfloat16),
            pltpu.VMEM((NS, PR, W), jnp.bfloat16),
            pltpu.VMEM((D, H * DH), jnp.bfloat16),
            pltpu.VMEM((H * DH, D), jnp.bfloat16),
            pltpu.VMEM((D, F), jnp.bfloat16),
            pltpu.VMEM((D, F), jnp.bfloat16),
            pltpu.VMEM((F, D), jnp.bfloat16),
            pltpu.VMEM((D, 6 * D), jnp.bfloat16),
            pltpu.VMEM((NP, M, PR), jnp.bfloat16),
            pltpu.SemaphoreType.DMA((NS,)),
            pltpu.SemaphoreType.DMA((NS,)),
            pltpu.SemaphoreType.DMA((5 + 3 * FCH,)),
        ],
        compiler_params=pltpu.CompilerParams(vmem_limit_bytes=100 * 1024 * 1024),
    )(x2, kt, vt, A_wq, A_wo, B_w_gate, B_w_up, B_w_down, c, w_mod)
    return out.reshape(A_x.shape)
```

```python
import contextlib
import functools
import jax
import jax.numpy as jnp
import numpy as np
import jax.experimental.pallas as pl
import jax.experimental.pallas.tpu as pltpu

D = 640
H = 32
DH = 192
F = 1536
M = 8
PR = 2 * DH
NP = H * DH // PR


def order_idx(nr, nc, order):
    if order == 'rc':
        idx = [(r, c) for r in range(nr) for c in range(nc)]
    elif order == 'cr':
        idx = [(r, c) for c in range(nc) for r in range(nr)]
    elif order == 'rc2':
        idx = [(r, c + h * (nc // 2)) for r in range(nr) for c in range(nc // 2) for h in range(2)]
    assert len(set(idx)) == nr * nc
    return idx


def make(NS=2, kv_blk=(16, 1024), kv_order='rc2', kv_loop=True,
         wm_blk=(32, 640), wq_blk=(16, 1024), wo_blk=(32, 640), gu_blk=(32, 512), wd_blk=(32, 640),
         d_chunks=(512, 512, 384, 128), prio=True, scopes=False, wo_pos='pair', compute=True):
    def scope(name):
        if scopes:
            return jax.named_scope(name)
        return contextlib.nullcontext()

    def kern(x_hbm, k_hbm, v_hbm, wq_hbm, wo_hbm, wg_hbm, wu_hbm, wd_hbm, c_hbm, wm_hbm,
             o_ref,
             x_v, c_v, kbuf, vbuf, wq_v, wo_v, wg_v, wu_v, wd_v, wm_v, q_s,
             ksem, vsem, osem, wsem, dsem):
        SK = k_hbm.shape[1]
        W = kbuf.shape[2]
        c0 = SK - W

        def issue(src, dst, sem, blk, order='rc', loop=True, sr0=None):
            nr_, nc_ = dst.shape[-2:]
            sr, sc = blk
            nr, nc = nr_ // sr, nc_ // sc
            assert nr * sr == nr_ and nc * sc == nc_, (dst.shape, blk)

            def one(r, c, pr):
                pltpu.make_async_copy(src.at[pl.ds(r, sr), pl.ds(c, sc)], dst.at[pl.ds(r, sr), pl.ds(c, sc)],
                                      sem).start(priority=pr if prio else 0)
            if not loop or nr == 1:
                for n, (r, c) in enumerate(order_idx(nr, nc, order)):
                    one(r * sr, c * sc, n % 2)
            else:
                assert order in ('rc', 'rc2')
                per = 1 if nc % 2 == 0 else 2
                assert nr % per == 0
                cols = [c for (_, c) in order_idx(1, nc, order)]

                def body(i, carry):
                    n = 0
                    for j in range(per):
                        r = pl.multiple_of((i * per + j) * sr, sr)
                        for c in cols:
                            one(r, c * sc, n % 2)
                            n += 1
                    return carry
                jax.lax.fori_loop(0, nr // per, body, 0)

        def wait(dst, sem):
            pltpu.make_async_copy(dst, dst, sem).wait()

        def issue_k(p, slot):
            issue(k_hbm.at[pl.ds(pl.multiple_of(p * PR, PR), PR), pl.ds(c0, W)], kbuf.at[slot], ksem.at[slot],
                  kv_blk, kv_order, kv_loop)

        def issue_v(p, slot):
            issue(v_hbm.at[pl.ds(pl.multiple_of(p * PR, PR), PR), pl.ds(c0, W)], vbuf.at[slot], vsem.at[slot],
                  kv_blk, kv_order, kv_loop)

        def issue_wo(p, slot):
            rows = pl.ds(pl.multiple_of(p * PR, PR), PR)
            issue(wo_hbm.at[rows], wo_v.at[slot], osem.at[slot], wo_blk, 'rc', False)

        c_cp = pltpu.make_async_copy(c_hbm, c_v, wsem.at[1])
        x_cp = pltpu.make_async_copy(x_hbm, x_v, wsem.at[0])
        d_off = [sum(d_chunks[:i]) for i in range(len(d_chunks))]

        c_cp.start()
        x_cp.start(priority=1 if prio else 0)
        issue(wm_hbm, wm_v, wsem.at[2], wm_blk)
        issue(wq_hbm, wq_v, wsem.at[3], wq_blk)

        c_cp.wait()
        cf = c_v[...].astype(jnp.float32)
        sc = cf * jax.nn.sigmoid(cf)
        sc = jnp.broadcast_to(sc, (M, D)).astype(jnp.bfloat16)
        wait(wm_v, wsem.at[2])
        mod = jnp.dot(sc, wm_v[...], preferred_element_type=jnp.float32)
        sa = mod[:, 0 * D:1 * D]
        ca = mod[:, 1 * D:2 * D]
        ga = mod[:, 2 * D:3 * D]
        sb = mod[:, 3 * D:4 * D]
        cb = mod[:, 4 * D:5 * D]
        gb = mod[:, 5 * D:6 * D]

        def ln(t):
            m = jnp.mean(t, axis=-1, keepdims=True)
            d = t - m
            v = jnp.mean(d * d, axis=-1, keepdims=True)
            return d * jax.lax.rsqrt(v + 1e-5)

        x_cp.wait()
        x = jnp.broadcast_to(x_v[...].astype(jnp.float32), (M, D))
        h = (ln(x) * (1.0 + ca) + sa).astype(jnp.bfloat16)

        issue_k(0, 0)
        wait(wq_v, wsem.at[3])
        row = jax.lax.broadcasted_iota(jnp.int32, (M, PR), 0)
        col = jax.lax.broadcasted_iota(jnp.int32, (M, PR), 1)
        hmask = ((row == 0) & (col < DH)) | ((row == 1) & (col >= DH))
        scale = DH ** -0.5
        for p in range(NP):
            q = jnp.dot(h, wq_v[:, p * PR:(p + 1) * PR], preferred_element_type=jnp.float32)
            q_s[p] = jnp.where(hmask, q * scale, 0.0).astype(jnp.bfloat16)
        issue_v(0, 0)
        issue_wo(0, 0)
        for s in range(1, NS):
            issue_k(s, s)
            issue_v(s, s)
            issue_wo(s, s)

        def body(p, acc):
            slot = p % NS
            wait(kbuf.at[slot], ksem.at[slot])
            s = jnp.dot(q_s[p], kbuf[slot], preferred_element_type=jnp.float32)
            m = jnp.max(s, axis=-1, keepdims=True)
            e = jnp.exp(s - m)
            l = jnp.sum(e, axis=-1, keepdims=True)
            eb = e.astype(jnp.bfloat16)

            @pl.when(p + NS < NP)
            def _():
                issue_k(p + NS, slot)

            @pl.when(p == NP - 1)
            def _():
                issue(wg_hbm, wg_v, wsem.at[4], gu_blk)
                issue(wu_hbm, wu_v, wsem.at[5], gu_blk)

            wait(vbuf.at[slot], vsem.at[slot])
            o = jax.lax.dot_general(eb, vbuf[slot], (((1,), (1,)), ((), ())),
                                    preferred_element_type=jnp.float32)
            on = jnp.where(hmask, o / l, 0.0).astype(jnp.bfloat16)
            wait(wo_v.at[slot], osem.at[slot])
            acc = acc + jnp.dot(on, wo_v[slot], preferred_element_type=jnp.float32)

            @pl.when(p + NS < NP)
            def _():
                issue_v(p + NS, slot)
                issue_wo(p + NS, slot)
            return acc

        acc = jax.lax.fori_loop(0, NP, body, jnp.zeros((M, D), jnp.float32))
        for i, n in enumerate(d_chunks):
            issue(wd_hbm.at[pl.ds(d_off[i], n)], wd_v.at[pl.ds(d_off[i], n)], dsem.at[i], wd_blk, 'rc', False)
        attn = jnp.sum(acc, axis=0, keepdims=True)
        x1 = x + ga * attn
        h2 = (ln(x1) * (1.0 + cb) + sb).astype(jnp.bfloat16)
        wait(wg_v, wsem.at[4])
        g = jnp.dot(h2, wg_v[...], preferred_element_type=jnp.float32)
        wait(wu_v, wsem.at[5])
        u = jnp.dot(h2, wu_v[...], preferred_element_type=jnp.float32)
        hh = (g * u).astype(jnp.bfloat16)
        y = jnp.zeros((M, D), jnp.float32)
        for i, n in enumerate(d_chunks):
            wait(wd_v.at[pl.ds(d_off[i], n)], dsem.at[i])
            y = y + jnp.dot(hh[:, d_off[i]:d_off[i] + n], wd_v[d_off[i]:d_off[i] + n, :], preferred_element_type=jnp.float32)
        out = x1 + gb * y
        o_ref[...] = out[0:1, :].astype(o_ref.dtype)

    @jax.jit
    def f(A_x, A_k_cache, A_v_cache, A_wq, A_wo, B_x, B_w_gate, B_w_up, B_w_down, c, w_mod):
        B, Hkv, SK, Dh = A_k_cache.shape
        W = min(4096, max(256, SK // 4))
        kt = jnp.transpose(A_k_cache, (0, 1, 3, 2)).reshape(Hkv * Dh, SK)
        vt = jnp.transpose(A_v_cache, (0, 1, 3, 2)).reshape(Hkv * Dh, SK)
        x2 = A_x.reshape(1, D)
        anyspec = pl.BlockSpec(memory_space=pl.ANY)
        out = pl.pallas_call(
            kern,
            in_specs=[anyspec] * 10,
            out_specs=pl.BlockSpec(memory_space=pltpu.VMEM),
            out_shape=jax.ShapeDtypeStruct((1, D), A_x.dtype),
            scratch_shapes=[
                pltpu.VMEM((1, D), jnp.bfloat16),
                pltpu.VMEM((1, D), jnp.bfloat16),
                pltpu.VMEM((NS, PR, W), jnp.bfloat16),
                pltpu.VMEM((NS, PR, W), jnp.bfloat16),
                pltpu.VMEM((D, H * DH), jnp.bfloat16),
                pltpu.VMEM((NS, PR, D), jnp.bfloat16),
                pltpu.VMEM((D, F), jnp.bfloat16),
                pltpu.VMEM((D, F), jnp.bfloat16),
                pltpu.VMEM((F, D), jnp.bfloat16),
                pltpu.VMEM((D, 6 * D), jnp.bfloat16),
                pltpu.VMEM((NP, M, PR), jnp.bfloat16),
                pltpu.SemaphoreType.DMA((NS,)),
                pltpu.SemaphoreType.DMA((NS,)),
                pltpu.SemaphoreType.DMA((NS,)),
                pltpu.SemaphoreType.DMA((6,)),
                pltpu.SemaphoreType.DMA((len(d_chunks),)),
            ],
            compiler_params=pltpu.CompilerParams(vmem_limit_bytes=100 * 1024 * 1024),
        )(x2, kt, vt, A_wq, A_wo, B_w_gate, B_w_up, B_w_down, c, w_mod)
        return out.reshape(A_x.shape)

    return f


pallas_adaLN_cond__sliding_block_cached__glu_gated_bilinear__decode_kernel = make()
```

```python
import contextlib
import functools
import jax
import jax.numpy as jnp
import numpy as np
import jax.experimental.pallas as pl
import jax.experimental.pallas.tpu as pltpu

D = 640
H = 32
DH = 192
F = 1536
M = 8
PR = 2 * DH
NP = H * DH // PR


def perm(n, mode):
    if mode == '' or n == 1:
        l = list(range(n))
    elif mode == '2':
        l = [i + h * (n // 2) for i in range(n // 2) for h in range(2)]
    elif mode == 'v':
        l = [x for i in range(n // 2) for x in (i, n - 1 - i)]
    elif mode == '3':
        l = [i + h * (n // 3) for i in range(n // 3) for h in range(3)]
    elif mode == '4':
        l = [i + h * (n // 4) for i in range(n // 4) for h in range(4)]
    assert sorted(l) == list(range(n)), (n, mode)
    return l


def make(NS=2, kv_blk=(32, 512, 'c2'),
         wm_blk=(32, 640, 'r2'), wq_blk=(16, 1024, 'r'), wo_blk=(32, 640, 'uc2'), gu_blk=(32, 512, 'r'), wd_blk=(32, 640, 'uc'),
         d_chunks=(512, 512, 384, 128), L=2, dpos=0, gpm='alt', upm='alt', dpm='alt', wo_all=None, prio=True, scopes=False, wo_pos='pair', compute=True):
    def scope(name):
        if scopes:
            return jax.named_scope(name)
        return contextlib.nullcontext()

    def kern(x_hbm, k_hbm, v_hbm, wq_hbm, wo_hbm, wg_hbm, wu_hbm, wd_hbm, c_hbm, wm_hbm,
             o_ref,
             x_v, c_v, kbuf, vbuf, wq_v, wo_v, wg_v, wu_v, wd_v, wm_v, q_s,
             ksem, vsem, osem, wsem, dsem):
        SK = k_hbm.shape[1]
        W = kbuf.shape[2]
        c0 = SK - W

        def issue(src, dst, sem, cfg, name='i', pm='alt'):
            sr, sc, order = cfg
            nr_, nc_ = dst.shape[-2:]
            nr, nc = nr_ // sr, nc_ // sc
            assert nr * sr == nr_ and nc * sc == nc_, (dst.shape, cfg)
            def prf(n):
                return (n % 2) if pm == 'alt' else ((n + 1) % 2 if pm == 'tla' else int(pm))
            unroll = order[0] == 'u'
            if unroll:
                order = order[1:]
            if order[0] == 'p':
                st = int(order[1:]); nb = nr * nc
                assert np.gcd(st, nb) == 1 and nb % 2 == 0, (st, nb)
                un = nb if (unroll or nb <= 4) else (4 if nb % 4 == 0 else 2)

                def pbody(t, carry):
                    for j in range(un):
                        idx = ((t * un + j) * st) % nb
                        r, c = (idx // nc) * sr, (idx % nc) * sc
                        if not isinstance(idx, int):
                            r, c = pl.multiple_of(r, sr), pl.multiple_of(c, sc)
                        pltpu.make_async_copy(src.at[pl.ds(r, sr), pl.ds(c, sc)], dst.at[pl.ds(r, sr), pl.ds(c, sc)],
                                              sem).start(priority=prf(j) if prio else 0)
                    return carry
                with scope(name):
                    if un == nb:
                        pbody(0, 0)
                    else:
                        jax.lax.fori_loop(0, nb // un, pbody, 0)
                return
            outer_r = order[0] == 'r'
            n_out, n_in = (nr, nc) if outer_r else (nc, nr)
            inner = perm(n_in, order[1:])

            def one(o, i, pr):
                r, c = (o, i * sc) if outer_r else (i * sr, o)
                pltpu.make_async_copy(src.at[pl.ds(r, sr), pl.ds(c, sc)], dst.at[pl.ds(r, sr), pl.ds(c, sc)],
                                      sem).start(priority=pr if prio else 0)
            so = sr if outer_r else sc
            with scope(name):
              if unroll or n_out == 1:
                n = 0
                for o in range(n_out):
                    for i in inner:
                        one(o * so, i, prf(n))
                        n += 1
              else:
                per = 1 if n_in % 2 == 0 else 2
                assert n_out % per == 0

                def body(t, carry):
                    n = 0
                    for j in range(per):
                        o = pl.multiple_of((t * per + j) * so, so)
                        for i in inner:
                            one(o, i, prf(n))
                            n += 1
                    return carry
                jax.lax.fori_loop(0, n_out // per, body, 0)

        def wait(dst, sem, name='w'):
            with scope(name):
                pltpu.make_async_copy(dst, dst, sem).wait()

        def issue_k(p, slot):
            issue(k_hbm.at[pl.ds(pl.multiple_of(p * PR, PR), PR), pl.ds(c0, W)], kbuf.at[slot], ksem.at[slot], kv_blk, 'i_k')

        def issue_v(p, slot):
            issue(v_hbm.at[pl.ds(pl.multiple_of(p * PR, PR), PR), pl.ds(c0, W)], vbuf.at[slot], vsem.at[slot], kv_blk, 'i_v')

        def issue_wo(p, slot):
            if wo_all is not None:
                return
            rows = pl.ds(pl.multiple_of(p * PR, PR), PR)
            issue(wo_hbm.at[rows], wo_v.at[slot], osem.at[slot], wo_blk, 'i_wo')

        c_cp = pltpu.make_async_copy(c_hbm, c_v, wsem.at[1])
        x_cp = pltpu.make_async_copy(x_hbm, x_v, wsem.at[0])
        d_off = [sum(d_chunks[:i]) for i in range(len(d_chunks))]

        c_cp.start()
        x_cp.start(priority=1 if prio else 0)
        issue(wm_hbm, wm_v, wsem.at[2], wm_blk, 'i_wm')
        issue(wq_hbm, wq_v, wsem.at[3], wq_blk, 'i_wq')

        c_cp.wait()
        cf = c_v[...].astype(jnp.float32)
        sc = cf * jax.nn.sigmoid(cf)
        sc = jnp.broadcast_to(sc, (M, D)).astype(jnp.bfloat16)
        wait(wm_v, wsem.at[2], 'w_wm')
        mod = jnp.dot(sc, wm_v[...], preferred_element_type=jnp.float32)
        sa = mod[:, 0 * D:1 * D]
        ca = mod[:, 1 * D:2 * D]
        ga = mod[:, 2 * D:3 * D]
        sb = mod[:, 3 * D:4 * D]
        cb = mod[:, 4 * D:5 * D]
        gb = mod[:, 5 * D:6 * D]

        def ln(t):
            m = jnp.mean(t, axis=-1, keepdims=True)
            d = t - m
            v = jnp.mean(d * d, axis=-1, keepdims=True)
            return d * jax.lax.rsqrt(v + 1e-5)

        x_cp.wait()
        x = jnp.broadcast_to(x_v[...].astype(jnp.float32), (M, D))
        h = (ln(x) * (1.0 + ca) + sa).astype(jnp.bfloat16)

        issue_k(0, 0)
        wait(wq_v, wsem.at[3], 'w_wq')
        row = jax.lax.broadcasted_iota(jnp.int32, (M, PR), 0)
        col = jax.lax.broadcasted_iota(jnp.int32, (M, PR), 1)
        hmask = ((row == 0) & (col < DH)) | ((row == 1) & (col >= DH))
        scale = DH ** -0.5
        for p in range(NP):
            q = jnp.dot(h, wq_v[:, p * PR:(p + 1) * PR], preferred_element_type=jnp.float32)
            q_s[p] = jnp.where(hmask, q * scale, 0.0).astype(jnp.bfloat16)
        issue_v(0, 0)
        issue_wo(0, 0)
        if wo_all is not None:
            issue(wo_hbm, wo_v, osem.at[0], wo_all, 'i_wo')
        if L == 2:
            issue_k(1, 1)

        def body(p, acc):
            slot = p % NS
            wait(kbuf.at[slot], ksem.at[slot], 'w_k')
            s = jnp.dot(q_s[p], kbuf[slot], preferred_element_type=jnp.float32)
            m = jnp.max(s, axis=-1, keepdims=True)
            e = jnp.exp(s - m)
            l = jnp.sum(e, axis=-1, keepdims=True)
            eb = e.astype(jnp.bfloat16)

            if L == 1:
                @pl.when(p + 1 < NP)
                def _():
                    issue_k(p + 1, (p + 1) % NS)

                @pl.when(p + 1 == NP)
                def _():
                    issue(wg_hbm, wg_v, wsem.at[4], gu_blk, 'i_g', gpm)
            else:
                @pl.when(p + 1 < NP)
                def _():
                    issue_v(p + 1, (p + 1) % NS)
                    issue_wo(p + 1, (p + 1) % NS)

                @pl.when(p + 1 == NP)
                def _():
                    issue(wu_hbm, wu_v, wsem.at[5], gu_blk, 'i_u', upm)

            wait(vbuf.at[slot], vsem.at[slot], 'w_v')
            o = jax.lax.dot_general(eb, vbuf[slot], (((1,), (1,)), ((), ())),
                                    preferred_element_type=jnp.float32)
            on = jnp.where(hmask, o / l, 0.0).astype(jnp.bfloat16)
            if wo_all is None:
                wait(wo_v.at[slot], osem.at[slot], 'w_wo')
                acc = acc + jnp.dot(on, wo_v[slot], preferred_element_type=jnp.float32)
            else:
                @pl.when(p == 0)
                def _():
                    wait(wo_v, osem.at[0], 'w_wo')
                acc = acc + jnp.dot(on, wo_v[pl.ds(pl.multiple_of(p * PR, PR), PR), :], preferred_element_type=jnp.float32)

            if L == 1:
                @pl.when(p + 1 < NP)
                def _():
                    issue_v(p + 1, (p + 1) % NS)
                    issue_wo(p + 1, (p + 1) % NS)

                @pl.when(p + 1 == NP)
                def _():
                    issue(wu_hbm, wu_v, wsem.at[5], gu_blk, 'i_u', upm)
            else:
                @pl.when(p + 2 < NP)
                def _():
                    issue_k(p + 2, slot)

                @pl.when(p + 2 == NP)
                def _():
                    issue(wg_hbm, wg_v, wsem.at[4], gu_blk, 'i_g', gpm)
            return acc

        acc = jax.lax.fori_loop(0, NP, body, jnp.zeros((M, D), jnp.float32))
        def issue_d():
            for i, n in enumerate(d_chunks):
                issue(wd_hbm.at[pl.ds(d_off[i], n)], wd_v.at[pl.ds(d_off[i], n)], dsem.at[i], wd_blk if not isinstance(wd_blk, list) else wd_blk[i], 'i_d', dpm if not isinstance(dpm, list) else dpm[i])
        if dpos == 0:
            issue_d()
        attn = jnp.sum(acc, axis=0, keepdims=True)
        x1 = x + ga * attn
        h2 = (ln(x1) * (1.0 + cb) + sb).astype(jnp.bfloat16)
        if dpos == 1:
            issue_d()
        wait(wg_v, wsem.at[4], 'w_g')
        g = jnp.dot(h2, wg_v[...], preferred_element_type=jnp.float32)
        if dpos == 2:
            issue_d()
        wait(wu_v, wsem.at[5], 'w_u')
        u = jnp.dot(h2, wu_v[...], preferred_element_type=jnp.float32)
        hh = (g * u).astype(jnp.bfloat16)
        y = jnp.zeros((M, D), jnp.float32)
        for i, n in enumerate(d_chunks):
            wait(wd_v.at[pl.ds(d_off[i], n)], dsem.at[i], 'w_d')
            y = y + jnp.dot(hh[:, d_off[i]:d_off[i] + n], wd_v[d_off[i]:d_off[i] + n, :], preferred_element_type=jnp.float32)
        out = x1 + gb * y
        o_ref[...] = out[0:1, :].astype(o_ref.dtype)

    @jax.jit
    def f(A_x, A_k_cache, A_v_cache, A_wq, A_wo, B_x, B_w_gate, B_w_up, B_w_down, c, w_mod):
        B, Hkv, SK, Dh = A_k_cache.shape
        W = min(4096, max(256, SK // 4))
        kt = jnp.transpose(A_k_cache, (0, 1, 3, 2)).reshape(Hkv * Dh, SK)
        vt = jnp.transpose(A_v_cache, (0, 1, 3, 2)).reshape(Hkv * Dh, SK)
        x2 = A_x.reshape(1, D)
        anyspec = pl.BlockSpec(memory_space=pl.ANY)
        out = pl.pallas_call(
            kern,
            in_specs=[anyspec] * 10,
            out_specs=pl.BlockSpec(memory_space=pltpu.VMEM),
            out_shape=jax.ShapeDtypeStruct((1, D), A_x.dtype),
            scratch_shapes=[
                pltpu.VMEM((1, D), jnp.bfloat16),
                pltpu.VMEM((1, D), jnp.bfloat16),
                pltpu.VMEM((NS, PR, W), jnp.bfloat16),
                pltpu.VMEM((NS, PR, W), jnp.bfloat16),
                pltpu.VMEM((D, H * DH), jnp.bfloat16),
                pltpu.VMEM((NS, PR, D) if wo_all is None else (H * DH, D), jnp.bfloat16),
                pltpu.VMEM((D, F), jnp.bfloat16),
                pltpu.VMEM((D, F), jnp.bfloat16),
                pltpu.VMEM((F, D), jnp.bfloat16),
                pltpu.VMEM((D, 6 * D), jnp.bfloat16),
                pltpu.VMEM((NP, M, PR), jnp.bfloat16),
                pltpu.SemaphoreType.DMA((NS,)),
                pltpu.SemaphoreType.DMA((NS,)),
                pltpu.SemaphoreType.DMA((NS,)),
                pltpu.SemaphoreType.DMA((6,)),
                pltpu.SemaphoreType.DMA((len(d_chunks),)),
            ],
            compiler_params=pltpu.CompilerParams(vmem_limit_bytes=100 * 1024 * 1024),
        )(x2, kt, vt, A_wq, A_wo, B_w_gate, B_w_up, B_w_down, c, w_mod)
        return out.reshape(A_x.shape)

    return f


pallas_adaLN_cond__sliding_block_cached__glu_gated_bilinear__decode_kernel = make(
    wq_blk=(16, 1024, 'p31'), wm_blk=(16, 1280, 'p23'), wo_all=(32, 640, 'p73'), gu_blk=(16, 768, 'p31'),
    wd_blk=[(32, 640, 'p7'), (32, 640, 'p7'), (32, 640, 'p5'), (32, 640, 'uc')], dpm='1')
```

```python
import jax
import jax.numpy as jnp
import jax.experimental.pallas as pl
import jax.experimental.pallas.tpu as pltpu

D = 640
H = 32
DH = 192
F = 1536
M = 8
PR = 2 * DH
NP = H * DH // PR
D_CHUNKS = (512, 512, 384, 128)


def _kernel(x_hbm, k_hbm, v_hbm, wq_hbm, wo_hbm, wg_hbm, wu_hbm, wd_hbm, c_hbm, wm_hbm,
            o_ref,
            x_v, c_v, kbuf, vbuf, wq_v, wo_v, wg_v, wu_v, wd_v, wm_v, q_s,
            ksem, vsem, wsem, dsem):
    SK = k_hbm.shape[1]
    W = kbuf.shape[2]
    c0 = SK - W

    def start(src, dst, sem, r, sr, c, sc, prio):
        pltpu.make_async_copy(src.at[pl.ds(r, sr), pl.ds(c, sc)], dst.at[pl.ds(r, sr), pl.ds(c, sc)],
                              sem).start(priority=prio)

    def issue_strided(src, dst, sem, sr, sc, stride, prio=None):
        nr, nc = dst.shape[0] // sr, dst.shape[1] // sc
        n = nr * nc
        assert n % 2 == 0 and nc & (nc - 1) == 0
        pr = (0, 1) if prio is None else (prio, prio)
        if n <= 16:
            for j in range(n):
                i = (j * stride) % n
                start(src, dst, sem, (i // nc) * sr, sr, (i % nc) * sc, sc, pr[j % 2])
            return

        def body(_, i):
            for j in range(2):
                start(src, dst, sem, pl.multiple_of((i // nc) * sr, sr), sr,
                      pl.multiple_of((i % nc) * sc, sc), sc, pr[j])
                i = i + stride
                i = jnp.where(i >= n, i - n, i)
            return i
        jax.lax.fori_loop(0, n // 2, body, jnp.int32(0))

    def issue_kv(src_hbm, buf, sem, p, slot):
        src = src_hbm.at[pl.ds(pl.multiple_of(p * PR, PR), PR), pl.ds(c0, W)]
        dst = buf.at[slot]
        nr = PR // 32
        rows = [r for i in range(nr // 2) for r in (i, nr - 1 - i)]

        def body(t, carry):
            c = pl.multiple_of(t * 512, 512)
            for j, r in enumerate(rows):
                start(src, dst, sem.at[slot], r * 32, 32, c, 512, j % 2)
            return carry
        jax.lax.fori_loop(0, W // 512, body, 0)

    def wait(dst, sem):
        pltpu.make_async_copy(dst, dst, sem).wait()

    c_cp = pltpu.make_async_copy(c_hbm, c_v, wsem.at[0])
    x_cp = pltpu.make_async_copy(x_hbm, x_v, wsem.at[1])
    c_cp.start()
    x_cp.start(priority=1)
    issue_strided(wm_hbm, wm_v, wsem.at[2], 8, 1920, 71)
    issue_strided(wq_hbm, wq_v, wsem.at[3], 8, 1536, 141)

    c_cp.wait()
    cf = c_v[...].astype(jnp.float32)
    sc = cf * jax.nn.sigmoid(cf)
    sc = jnp.broadcast_to(sc, (M, D)).astype(jnp.bfloat16)
    wait(wm_v, wsem.at[2])
    mod = jnp.dot(sc, wm_v[...], preferred_element_type=jnp.float32)
    sa, ca, ga, sb, cb, gb = (mod[:, i * D:(i + 1) * D] for i in range(6))

    def ln(t):
        m = jnp.mean(t, axis=-1, keepdims=True)
        d = t - m
        v = jnp.mean(d * d, axis=-1, keepdims=True)
        return d * jax.lax.rsqrt(v + 1e-5)

    x_cp.wait()
    x = jnp.broadcast_to(x_v[...].astype(jnp.float32), (M, D))
    h = (ln(x) * (1.0 + ca) + sa).astype(jnp.bfloat16)

    issue_kv(k_hbm, kbuf, ksem, 0, 0)
    wait(wq_v, wsem.at[3])
    row = jax.lax.broadcasted_iota(jnp.int32, (M, PR), 0)
    col = jax.lax.broadcasted_iota(jnp.int32, (M, PR), 1)
    hmask = ((row == 0) & (col < DH)) | ((row == 1) & (col >= DH))
    scale = DH ** -0.5
    for p in range(NP):
        q = jnp.dot(h, wq_v[:, p * PR:(p + 1) * PR], preferred_element_type=jnp.float32)
        q_s[p] = jnp.where(hmask, q * scale, 0.0).astype(jnp.bfloat16)
    issue_kv(v_hbm, vbuf, vsem, 0, 0)
    issue_strided(wo_hbm, wo_v, wsem.at[4], 32, D, 73)
    issue_kv(k_hbm, kbuf, ksem, 1, 1)

    def body(p, acc):
        slot = p % 2
        wait(kbuf.at[slot], ksem.at[slot])
        s = jnp.dot(q_s[p], kbuf[slot], preferred_element_type=jnp.float32)
        m = jnp.max(s, axis=-1, keepdims=True)
        e = jnp.exp(s - m)
        l = jnp.sum(e, axis=-1, keepdims=True)
        eb = e.astype(jnp.bfloat16)

        @pl.when(p + 1 < NP)
        def _():
            issue_kv(v_hbm, vbuf, vsem, p + 1, (p + 1) % 2)

        @pl.when(p + 1 == NP)
        def _():
            issue_strided(wu_hbm, wu_v, wsem.at[6], 8, F, 11)

        wait(vbuf.at[slot], vsem.at[slot])
        o = jax.lax.dot_general(eb, vbuf[slot], (((1,), (1,)), ((), ())),
                                preferred_element_type=jnp.float32)
        on = jnp.where(hmask, o / l, 0.0).astype(jnp.bfloat16)

        @pl.when(p == 0)
        def _():
            wait(wo_v, wsem.at[4])
        acc = acc + jnp.dot(on, wo_v[pl.ds(pl.multiple_of(p * PR, PR), PR), :],
                            preferred_element_type=jnp.float32)

        @pl.when(p + 2 < NP)
        def _():
            issue_kv(k_hbm, kbuf, ksem, p + 2, slot)

        @pl.when(p + 2 == NP)
        def _():
            issue_strided(wg_hbm, wg_v, wsem.at[5], 8, F, 11)
        return acc

    acc = jax.lax.fori_loop(0, NP, body, jnp.zeros((M, D), jnp.float32))

    d_off = [sum(D_CHUNKS[:i]) for i in range(len(D_CHUNKS))]
    for i, n in enumerate(D_CHUNKS):
        issue_strided(wd_hbm.at[pl.ds(d_off[i], n)], wd_v.at[pl.ds(d_off[i], n)], dsem.at[i],
                      32, D, (7, 7, 5, 1)[i], prio=1)
    attn = jnp.sum(acc, axis=0, keepdims=True)
    x1 = x + ga * attn
    h2 = (ln(x1) * (1.0 + cb) + sb).astype(jnp.bfloat16)
    wait(wg_v, wsem.at[5])
    g = jnp.dot(h2, wg_v[...], preferred_element_type=jnp.float32)
    wait(wu_v, wsem.at[6])
    u = jnp.dot(h2, wu_v[...], preferred_element_type=jnp.float32)
    hh = (g * u).astype(jnp.bfloat16)
    y = jnp.zeros((M, D), jnp.float32)
    for i, n in enumerate(D_CHUNKS):
        wait(wd_v.at[pl.ds(d_off[i], n)], dsem.at[i])
        y = y + jnp.dot(hh[:, d_off[i]:d_off[i] + n], wd_v[d_off[i]:d_off[i] + n, :],
                        preferred_element_type=jnp.float32)
    out = x1 + gb * y
    o_ref[...] = out[0:1, :].astype(o_ref.dtype)


@jax.jit
def pallas_adaLN_cond__sliding_block_cached__glu_gated_bilinear__decode_kernel(
    A_x: jax.Array,
    A_k_cache: jax.Array,
    A_v_cache: jax.Array,
    A_wq: jax.Array,
    A_wo: jax.Array,
    B_x: jax.Array,
    B_w_gate: jax.Array,
    B_w_up: jax.Array,
    B_w_down: jax.Array,
    c: jax.Array,
    w_mod: jax.Array,
):
    B, Hkv, SK, Dh = A_k_cache.shape
    W = min(4096, max(256, SK // 4))
    kt = jnp.transpose(A_k_cache, (0, 1, 3, 2)).reshape(Hkv * Dh, SK)
    vt = jnp.transpose(A_v_cache, (0, 1, 3, 2)).reshape(Hkv * Dh, SK)
    x2 = A_x.reshape(1, D)
    anyspec = pl.BlockSpec(memory_space=pl.ANY)
    out = pl.pallas_call(
        _kernel,
        in_specs=[anyspec] * 10,
        out_specs=pl.BlockSpec(memory_space=pltpu.VMEM),
        out_shape=jax.ShapeDtypeStruct((1, D), A_x.dtype),
        scratch_shapes=[
            pltpu.VMEM((1, D), jnp.bfloat16),
            pltpu.VMEM((1, D), jnp.bfloat16),
            pltpu.VMEM((2, PR, W), jnp.bfloat16),
            pltpu.VMEM((2, PR, W), jnp.bfloat16),
            pltpu.VMEM((D, H * DH), jnp.bfloat16),
            pltpu.VMEM((H * DH, D), jnp.bfloat16),
            pltpu.VMEM((D, F), jnp.bfloat16),
            pltpu.VMEM((D, F), jnp.bfloat16),
            pltpu.VMEM((F, D), jnp.bfloat16),
            pltpu.VMEM((D, 6 * D), jnp.bfloat16),
            pltpu.VMEM((NP, M, PR), jnp.bfloat16),
            pltpu.SemaphoreType.DMA((2,)),
            pltpu.SemaphoreType.DMA((2,)),
            pltpu.SemaphoreType.DMA((7,)),
            pltpu.SemaphoreType.DMA((len(D_CHUNKS),)),
        ],
        compiler_params=pltpu.CompilerParams(vmem_limit_bytes=100 * 1024 * 1024),
    )(x2, kt, vt, A_wq, A_wo, B_w_gate, B_w_up, B_w_down, c, w_mod)
    return out.reshape(A_x.shape)
```
